```python
import os as _os
_os.environ.setdefault("JAX_PLATFORMS", "cpu")
import jax
import jax.numpy as jnp

def _softmax(x, axis=-1):
    return jax.nn.softmax(x, axis=axis)
def _gelu(x):
    return jax.nn.gelu(x, approximate=True)
def _silu(x):
    return jax.nn.silu(x)
def _sigmoid(x):
    return jax.nn.sigmoid(x)
def _layernorm(x, axis=-1, eps=1e-5):
    m = jnp.mean(x, axis=axis, keepdims=True)
    v = jnp.var(x, axis=axis, keepdims=True)
    return (x - m) / jnp.sqrt(v + eps)
def _scatter_add(tgt, idx, src, axis=0):
    return tgt.at[idx].add(src)
def _segment_sum(src, seg, n):
    return jax.ops.segment_sum(src, seg, n)
class _Rng:
    def __init__(self, key):
        self._k = key
    def _next(self):
        self._k, sub = jax.random.split(self._k)
        return sub
    def normal(self, shape):
        return jax.random.normal(self._next(), shape, dtype=jnp.bfloat16)
    def randint(self, lo, hi, shape):
        return jax.random.randint(self._next(), shape, lo, hi, dtype=jnp.int32)
    def uniform(self, shape, lo=0.0, hi=1.0):
        return jax.random.uniform(self._next(), shape, jnp.bfloat16, lo, hi)
    def permutation(self, n):
        return jax.random.permutation(self._next(), n)


kernel_name = 'gated_mix__grouped_kv_mqa__glu_gated_reglu__prompt'

def setup_inputs():
    _rng = _Rng(jax.random.key(int.from_bytes(__import__("os").urandom(4), "little")))
    _w = (lambda a: (lambda t: t.astype(jnp.bfloat16) if jnp.issubdtype(t.dtype, jnp.floating) else t)(jnp.asarray(a)))
    def _A_setup():
        B, S, D, H = 1, 2048, 1024, 32
        Dh = D // H
        return {
            "x": _w((lambda *s: _rng.normal(s) * 0.05)(B, S, D)),
            "wq": _w((lambda *s: _rng.normal(s) * 0.2)(D, H * Dh)),
            "wk": _w((lambda *s: _rng.normal(s) * 0.2)(D, Dh)),
            "wv": _w((lambda *s: _rng.normal(s) * 0.05)(D, Dh)),
            "wo": _w((lambda *s: _rng.normal(s) * 0.05)(H * Dh, D)),
        }
    _A_in = _A_setup()

    def _B_setup():
        B, S, D, F = 1, 2048, 1024, 3584
        return {
            "x": _w((lambda *s: _rng.normal(s) * 0.05)(B, S, D)),
            "W_gate": _w((lambda *s: _rng.normal(s) * 0.8)(D, F) * (2.0 / D) ** 0.5),
            "W_up": _w((lambda *s: _rng.normal(s) * 0.8)(D, F) * (2.0 / D) ** 0.5),
            "W_down": _w((lambda *s: _rng.normal(s) * 0.8)(F, D) * (1.0 / F) ** 0.5),
        }
    _B_in = _B_setup()

    return {
        "A_x": _A_in["x"],
        "A_wq": _A_in["wq"],
        "A_wk": _A_in["wk"],
        "A_wv": _A_in["wv"],
        "A_wo": _A_in["wo"],
        "B_x": _B_in["x"],
        "B_W_gate": _B_in["W_gate"],
        "B_W_up": _B_in["W_up"],
        "B_W_down": _B_in["W_down"],
        "gate_w": _w((lambda *s: _rng.normal(s) * 0.05)(1024) * 16.0),
    }

def reference(A_x, A_wq, A_wk, A_wv, A_wo, B_x, B_W_gate, B_W_up, B_W_down, gate_w):
    def _A_ref(x, wq, wk, wv, wo):
        B, S, D = x.shape
        H = 32
        Dh = D // H
        q = (lambda x, *d: x.transpose(*d))((x @ wq).reshape(B, S, H, Dh), 0, 2, 1, 3)
        k = x @ wk
        v = x @ wv
        scores = jnp.einsum("bhqd,bkd->bhqk", q, k) * (Dh ** -0.5)
        p = _softmax(scores, axis=-1)
        o = jnp.einsum("bhqk,bkd->bhqd", p, v)
        return (lambda x, *d: x.transpose(*d))(o, 0, 2, 1, 3).reshape(B, S, H * Dh) @ wo

    def _B_ref(x, W_gate, W_up, W_down):
        gate = jnp.einsum("bsd,df->bsf", x, W_gate)
        up = jnp.einsum("bsd,df->bsf", x, W_up)
        gate = gate * (lambda x, dt: x.astype(dt))(gate > 0, gate.dtype)
        h = gate * up
        return jnp.einsum("bsf,fd->bsd", h, W_down)

    x = A_x
    g = _sigmoid((x * gate_w).sum(-1, keepdims=True))
    a = _A_ref(x, A_wq, A_wk, A_wv, A_wo)
    b = _B_ref(x, B_W_gate, B_W_up, B_W_down)
    return g * a + (1 - g) * b
```

```python
import math

import jax
import jax.numpy as jnp
from jax import lax
import jax.experimental.pallas as pl
import jax.experimental.pallas.tpu as pltpu

F32 = jnp.float32
BF16 = jnp.bfloat16

S, D, H, DH, F = 2048, 1024, 32, 32, 3584
TQ = 512
KC = 128
HG = 4
NR = S // TQ
NG = H // HG
TM = 256
FC = 512

_NT = (((1,), (1,)), ((), ()))


def _fold8(x, op):
    parts = [x[i:i + 8] for i in range(0, x.shape[0], 8)]
    while len(parts) > 1:
        parts = [op(parts[i], parts[i + 1]) if i + 1 < len(parts) else parts[i]
                 for i in range(0, len(parts), 2)]
    return parts[0]


def _dot(a, b):
    return jnp.dot(a, b, preferred_element_type=F32)


def _kernel(x_hbm, wq_hbm, wkt_ref, wvt_ref, wo_hbm, wg_hbm, wu_hbm, wd_hbm, gw_ref,
            out_hbm,
            x_v, wq_v, wo_v, wg_v, wu_v, wd_v,
            k_s, vt_s, qt_s, gt_s, gc_s, s_buf, o_s, h_s, out_v,
            x_sem, w_sem, o_sem):
    x_copies = [pltpu.make_async_copy(x_hbm.at[pl.ds(r * TQ, TQ)], x_v.at[pl.ds(r * TQ, TQ)],
                                      x_sem.at[r]) for r in range(NR)]
    w_copies = [pltpu.make_async_copy(src, dst, w_sem.at[i]) for i, (src, dst) in enumerate(
        ((wq_hbm, wq_v), (wg_hbm, wg_v), (wu_hbm, wu_v), (wd_hbm, wd_v), (wo_hbm, wo_v)))]
    x_copies[0].start()
    w_copies[0].start()
    for c in x_copies[1:]:
        c.start()

    qk_scale = DH ** -0.5 * math.log2(math.e)
    wkvg = jnp.concatenate(
        [wkt_ref[...], wvt_ref[...], jnp.broadcast_to(gw_ref[...], (16, D))], axis=0)
    for r in range(NR):
        x_copies[r].wait()
        xr = x_v[r * TQ:(r + 1) * TQ, :]
        kvg = lax.dot_general(wkvg, xr, _NT, preferred_element_type=F32)
        vt_s[:, r * TQ:(r + 1) * TQ] = kvg[32:64].astype(BF16)
        g = jax.nn.sigmoid(kvg[64:72])
        gt_s[r] = g
        tr = jnp.concatenate(
            [kvg[0:32] * qk_scale, 1.0 - g, jnp.zeros((88, TQ), F32)], axis=0).T
        k_s[r * TQ:(r + 1) * TQ, :] = tr[:, 0:32].astype(BF16)
        gc_s[r * TQ:(r + 1) * TQ, :] = jnp.broadcast_to(tr[:, 32:33], (TQ, 128))
        if r == 0:
            w_copies[0].wait()
            for c in w_copies[1:]:
                c.start()
        q = _dot(xr, wq_v[...])
        qt_s[r * D:(r + 1) * D, :] = q.T.astype(BF16)

    def qk_chunk(c, qt, m8):
        s = _dot(k_s[c * KC:(c + 1) * KC, :], qt)
        s_buf[c * KC:(c + 1) * KC, :] = s
        t = _fold8(s, jnp.maximum)
        return t if m8 is None else jnp.maximum(m8, t)

    def head(m, qt_next):
        acc = l8 = m8 = None
        for c in range(S // KC):
            p = jnp.exp2(s_buf[c * KC:(c + 1) * KC, :] - m)
            t = _fold8(p, jnp.add)
            l8 = t if l8 is None else l8 + t
            o = _dot(vt_s[:, c * KC:(c + 1) * KC], p.astype(BF16))
            acc = o if acc is None else acc + o
            if qt_next is not None:
                m8 = qk_chunk(c, qt_next, m8)
        l = jnp.sum(l8, axis=0, keepdims=True)
        m_next = None if m8 is None else jnp.max(m8, axis=0, keepdims=True)
        return acc, l, m_next

    m8 = None
    qt0 = qt_s[0:DH, :]
    for c in range(S // KC):
        m8 = qk_chunk(c, qt0, m8)
    m0 = jnp.max(m8, axis=0, keepdims=True)

    def group(i, m):
        r = i // NG
        g = gt_s[r][0:1]
        outs = []
        for j in range(HG):
            nxt = jnp.minimum(i * HG + j + 1, NR * H - 1)
            qt_next = qt_s[pl.ds(pl.multiple_of(nxt * DH, DH), DH), :]
            acc, l, m = head(m, qt_next)
            outs.append(acc * (g / l))
        o = jnp.concatenate(outs, axis=0).T
        o_s[i % NG, pl.ds(pl.multiple_of(r * TQ, TQ), TQ), :] = o.astype(BF16)
        return m

    lax.fori_loop(0, NR * NG, group, m0)

    for c in w_copies[1:]:
        c.wait()

    def out_copy(i, slot):
        return pltpu.make_async_copy(
            out_v.at[slot], out_hbm.at[pl.ds(pl.multiple_of(i * TM, TM), TM)], o_sem.at[slot])

    def ffn(i, carry):
        rows = pl.ds(pl.multiple_of(i * TM, TM), TM)
        slot = i % 2
        xr = x_v[rows, :]
        gc = gc_s[rows, :]
        for f in range(F // FC):
            gate = _dot(xr, wg_v[:, f * FC:(f + 1) * FC])
            up = _dot(xr, wu_v[:, f * FC:(f + 1) * FC])
            hh = jnp.maximum(gate, 0.0) * up
            h_s[:, f * FC:(f + 1) * FC] = hh.astype(BF16)
        b = _dot(h_s[...], wd_v[...])
        o = jnp.concatenate([o_s[j, rows, :] for j in range(NG)], axis=1)
        a = _dot(o, wo_v[...])
        res = a + b * jnp.concatenate([gc] * (D // 128), axis=1)

        @pl.when(i >= 2)
        def _():
            out_copy(i - 2, slot).wait()

        out_v[slot] = res.astype(BF16)
        out_copy(i, slot).start()
        return carry

    n = S // TM
    lax.fori_loop(0, n, ffn, 0)
    out_copy(n - 2, (n - 2) % 2).wait()
    out_copy(n - 1, (n - 1) % 2).wait()


@jax.jit
def pallas_gated_mix__grouped_kv_mqa__glu_gated_reglu__prompt_kernel(
        A_x, A_wq, A_wk, A_wv, A_wo, B_x, B_W_gate, B_W_up, B_W_down, gate_w):
    del B_x
    hbm = pl.BlockSpec(memory_space=pl.ANY)
    vmem = pl.BlockSpec(memory_space=pltpu.VMEM)
    out = pl.pallas_call(
        _kernel,
        out_shape=jax.ShapeDtypeStruct((S, D), BF16),
        in_specs=[hbm, hbm, vmem, vmem, hbm, hbm, hbm, hbm, vmem],
        out_specs=hbm,
        scratch_shapes=[
            pltpu.VMEM((S, D), BF16), pltpu.VMEM((D, D), BF16), pltpu.VMEM((D, D), BF16),
            pltpu.VMEM((D, F), BF16), pltpu.VMEM((D, F), BF16), pltpu.VMEM((F, D), BF16),
            pltpu.VMEM((S, DH), BF16), pltpu.VMEM((DH, S), BF16), pltpu.VMEM((NR * D, TQ), BF16),
            pltpu.VMEM((NR, 8, TQ), F32), pltpu.VMEM((S, 128), F32),
            pltpu.VMEM((S, TQ), F32), pltpu.VMEM((NG, S, 128), BF16),
            pltpu.VMEM((TM, F), BF16), pltpu.VMEM((2, TM, D), BF16),
            pltpu.SemaphoreType.DMA((NR,)), pltpu.SemaphoreType.DMA((5,)),
            pltpu.SemaphoreType.DMA((2,)),
        ],
        compiler_params=pltpu.CompilerParams(vmem_limit_bytes=110 * 2 ** 20),
        name="gated_mix",
    )(A_x.reshape(S, D), A_wq, A_wk.T, A_wv.T, A_wo, B_W_gate, B_W_up, B_W_down,
      gate_w.reshape(1, D))
    return out.reshape(1, S, D)
```

```python
import math

import jax
import jax.numpy as jnp
from jax import lax
import jax.experimental.pallas as pl
import jax.experimental.pallas.tpu as pltpu

F32 = jnp.float32
BF16 = jnp.bfloat16
U32 = jnp.uint32

S, D, H, DH, F = 2048, 1024, 32, 32, 3584
T = 128
NT = S // T
CH = 4 * T
NCH = S // CH
NQ = F // CH
NP = 49

VECTOR_KEYS = 112
STEP_PLAN = (("DDDDRL", -3.185, -0.2), ("URRR", 0, 0.831), ("G", 1.085, 1.961),
             ("HLLL", 2.025, 3.0))
TRANSPOSE_LAG = 0.224
OPERAND_COST = 320

_LEFT = (((0, 0, 1), (1, 1, -1)), ((1, 0, 1), (1, 1, -1)), ((0, 0, 1),), ((1, 1, 1),),
         ((0, 0, 1), (0, 1, -1)), ((1, 0, 1), (0, 0, -1)), ((1, 1, 1), (0, 1, -1)))
_RIGHT = (((0, 0, 1), (1, 1, -1)), ((0, 0, 1),), ((0, 1, 1), (1, 1, 1)), ((1, 0, 1), (0, 0, 1)),
          ((1, 1, 1),), ((0, 0, 1), (0, 1, 1)), ((1, 0, 1), (1, 1, 1)))
_RESULT = (((0, 0, 1), (1, 1, 1)), ((1, 0, 1), (1, 1, -1)), ((0, 1, 1), (1, 1, 1)),
           ((0, 0, 1), (1, 0, 1)), ((0, 0, 1), (0, 1, -1)), ((1, 1, 1),), ((0, 0, -1),))
_ORDER = (0, 3, 1, 2, 5, 4, 6)
_LAST = {(i, j): u for u in _ORDER for i, j, _ in _RESULT[u]}


def _dot(a, b):
    return jnp.dot(a, b, preferred_element_type=F32)


def _pack(x):
    return pltpu.bitcast(x.astype(BF16), U32)


def _unpack(x):
    return pltpu.bitcast(x, BF16)


def _rows(i, n):
    return pl.ds(i * n, n) if isinstance(i, int) else pl.ds(pl.multiple_of(i * n, n), n)


def _zero(i):
    return ((i * (i + 1)) & 1) * (i * 7777 - 99999)


def _signed_sum(terms):
    total = None
    for v, sign in terms:
        total = v if total is None else (total + v if sign > 0 else total - v)
    return total


def _operands(coef, block, emit):
    for u in range(7):
        v = {(i, j): _signed_sum([(block(2 * bi + i, 2 * bj + j), s) for bi, bj, s in coef[u]])
             for i in (0, 1) for j in (0, 1)}
        for w in range(7):
            emit(7 * u + w, _signed_sum([(v[i, j], s) for i, j, s in coef[w]]))
        yield


def _combine(product, emit):
    out = {}
    for u in _ORDER:
        m = [product(7 * u + w) for w in range(7)]
        c = {(0, 0): (m[0] + m[3]) + (m[4] - m[6]), (0, 1): m[2] - m[4],
             (1, 0): m[1] + m[3], (1, 1): (m[0] - m[1]) + (m[2] + m[5])}
        for bi, bj, sign in _RESULT[u]:
            for (i, j), v in c.items():
                key = (2 * bi + i, 2 * bj + j)
                out[key] = v if key not in out else (out[key] + v if sign > 0 else out[key] - v)
                if _LAST[bi, bj] == u:
                    emit(*key, out[key])
        yield


def _fold(x, op, total):
    for lo in range(0, x.shape[0], 32):
        parts = [x[i:i + 8] for i in range(lo, min(lo + 32, x.shape[0]), 8)]
        while len(parts) > 1:
            parts = [op(*parts[i:i + 2]) if i + 1 < len(parts) else parts[i]
                     for i in range(0, len(parts), 2)]
        total = parts[0] if total is None else op(total, parts[0])
    return total


def _whole(gen):
    for _ in gen:
        pass
    yield


class _Job:
    def __init__(self, gen, steps, cost, src, dst, lag=None, made=None):
        self.gen, self.steps, self.cost, self.src, self.dst = gen, steps, cost, src, dst
        self.lag, self.made = lag, made


class _Block:
    def __init__(self, zero, lag=0.106):
        self.zero, self.lag, self.now = zero, lag, 0.0
        self.events, self.results, self.feeds, self.index = [], [], [], {}

    def at(self, t, gen, job=None):
        self.events.append((t, len(self.events), gen, job))

    def matmuls(self, gen, steps, lo, hi, feed=None):
        for k in range(steps):
            self.at(lo + (hi - lo) * k / steps, gen)
        if feed is not None:
            self.feeds.append((lo, hi, feed))

    def jobs(self, lo, hi, *lists):
        order = sorted(((k + 0.5) / len(js), n, k)
                       for n, js in enumerate(lists) for k in range(len(js)))
        merged = [lists[n][k] for _, n, k in order]
        unit = (hi - lo) / max(sum(job.cost for job in merged), 1)
        for job in merged:
            span = unit * job.cost
            for k in range(job.steps):
                t = lo + span * (k + 0.5) / job.steps
                self.at(t, job.gen, job)
            if job.dst:
                gen = self.deadline(job)
                self.at(t, gen)
                self.at(t + (job.lag or self.lag), gen)
            lo += span

    def note(self, result, duration, lag=0.0):
        n = result.shape[0] // 8
        self.results += [(self.now + lag + duration * (k + 1) / n, result, 8 * k)
                         for k in range(n)]

    def unused(self, where):
        buf, *lead, tile = where
        if tile not in self.index:
            self.index[tile] = tile + self.zero
        return buf, (*lead, self.index[tile], slice(buf.shape[-2] - 8, buf.shape[-2]), slice(0, T))

    def put(self, where, v):
        buf, rows = self.unused(where)
        v = lax.bitcast_convert_type(v, F32) if v.dtype == U32 else v.astype(F32)
        buf[rows] = lax.bitcast_convert_type(v, U32) if buf.dtype == U32 else v.astype(buf.dtype)

    def recent(self, t):
        found = next((r for r in reversed(self.results) if r[0] <= t), None)
        return found and found[1][found[2]:found[2] + 8, 0:T]

    def barrier(self, where, timed=False):
        v = self.recent(self.now - self.lag) if timed else None
        self.put(where, jnp.full((8, T), self.now, F32) if v is None else v)

    def deadline(self, job):
        buf, rows = self.unused(job.dst)
        v = buf[rows]
        yield
        for lo, hi, feed in self.feeds:
            if lo <= self.now < hi:
                self.put(feed, v)
        yield

    def run(self):
        for t, _, gen, job in sorted(self.events, key=lambda e: e[:2]):
            self.now = t
            v = job and self.recent(t)
            if v is not None:
                if job.made is not None and len(job.made) >= 2:
                    v = v + job.made[-2][0:8]
                self.put(job.src, v)
            v = next(gen)
            if v is not None:
                job.made.append(v)


def _start(copies):
    for copy in copies:
        copy.start()


def _wait(copies):
    for copy in copies:
        copy.wait()


def _kernel(x_hbm, wq_hbm, wkt_hbm, wvt_hbm, wo_hbm, wg_hbm, wu_hbm, wd_hbm, gw_hbm, out_hbm,
            raw, xa, wl, wr, wd, rl, rr, g_buf, h_buf, ha, acc,
            k_s, vt_s, gt_s, gc_s, qt_s, m_s, ot_s, qo_s, s_buf, kb_s, qb_s, x_v, wkv, gw_v,
            x_sem, w_sem, sem):
    raw_spare = (raw, 8)

    def side_copies(quad, square=None):
        if square is None:
            srcs, first = [w.at[:, _rows(quad - 1, CH)] for w in (wg_hbm, wu_hbm)], 2
        else:
            srcs, first = [square.at[:, pl.ds(side * CH, CH)] for side in (0, 1)], 0
        return [pltpu.make_async_copy(src, raw.at[2 * (quad & 1) + side], w_sem.at[first + side])
                for side, src in enumerate(srcs)]

    def down_copies(quad):
        return [pltpu.make_async_copy(wd_hbm.at[_rows(quad - 1, CH), pl.ds(side * CH, CH)],
                                      raw.at[4 + (quad & 3), pl.ds(side * CH, CH)],
                                      w_sem.at[4 + side])
                for side in (0, 1)]

    def side_operands(side, quad, first, count):
        w, slot = (wl, wr)[side], quad & 1
        src = 2 * slot + side

        def job(pos):
            k, rows = pos >> 3, _rows(pos & 7, 8)
            blocks = [_rows(a * 16 + pos, 16) for a in range(4)]

            def emit(t, v):
                w[slot, 2 * t + k, rows, :] = _pack(v)

            def block(a, b):
                return raw[src, blocks[a], b * T:(b + 1) * T].astype(F32)

            return _Job(_operands(_RIGHT, block, emit), 7, OPERAND_COST, raw_spare, (w, 0, 2 * NP))
        return [job(first + p) for p in range(count)]

    def down_operands(source, quad, first, count):
        slot, src = quad & 1, 4 + (source & 3)

        def job(pos, side):
            rows = _rows(pos, 8)
            blocks = [_rows(side * 32 + a * 8 + pos, 16) for a in range(4)]

            def emit(t, v):
                wd[slot, 2 * t + side, rows, :] = _pack(v)

            def block(a, b):
                return raw[src, blocks[a], b * T:(b + 1) * T].astype(F32)

            return _Job(_operands(_RIGHT, block, emit), 7, OPERAND_COST, raw_spare, (wd, 0, 2 * NP))
        return [job(first + p // 2, p % 2) for p in range(count)]

    def row_operands(c, block, src, cost):
        def job(j, k):
            def emit(t, v):
                xa[2 * t + k, _rows(c * 8 + j, 8), :] = _pack(v)

            return _Job(_operands(_LEFT, lambda a, b: block(a, 2 * b + k, j), emit), 7, cost, src,
                        (xa, 2 * NP))
        return [job(j, k) for j in range(T // 16) for k in (0, 1)]

    def products(blk, side, quad, c, lo, again=False, base=None, out=None):
        w, r = (wl, wr)[side], (rl, rr)[side if out is None else out]
        slot, rows = quad & 1, _rows(c, T // 2)

        def gen():
            if again:
                blk.barrier((xa, 2 * NP),
                            isinstance(c, int) and c == NCH - 1 and quad in (0, NQ + 1))
            for t in range(NP):
                a = jnp.concatenate([_unpack(xa[2 * t + k, rows, :]) for k in (0, 1)], axis=1)
                b = jnp.concatenate([_unpack(w[slot, 2 * t + k, 0:T // 2, :]) for k in (0, 1)],
                                    axis=0)
                res = _dot(a, b)
                if base is not None:
                    res = res + base(t)
                r[t, 0:T, :] = res
                if t % 2 == 0:
                    blk.note(res, 2 / NP)
                yield
        blk.matmuls(gen(), NP, lo, lo + 1, (w, 0, 2 * NP))

    def results(r, finish, dst):
        def job(rows):
            return _Job(_combine(lambda t: r[t, rows, :], lambda a, b, v: finish(a, b, rows, v)),
                        7, 130, (r, NP), dst)
        return [job(slice(8 * j, 8 * j + 8)) for j in range(T // 8)]

    def scores(blk, h, lo, hi, width, later=0):
        edges = [(S - later) // 16 * k // NT * 16 for k in range(NT + 1)]
        steps = NT // width * NT

        def gen():
            for first in range(0, NT, width):
                tiles = range(first, first + width)
                q = jnp.concatenate([qt_s[i, _rows(h & 15, DH), :] for i in tiles], axis=1)
                m = None
                for k0, k1 in zip(edges, edges[1:]):
                    s = _dot(_unpack(k_s[k0 // 2:k1 // 2, :])[:, 0:DH], q)
                    yield
                    for j, i in enumerate(tiles):
                        s_buf[i, k0:k1, :] = s[:, j * T:(j + 1) * T]
                    m = _fold(s, jnp.maximum, m)
                    blk.note(s[0:(k1 - k0) * width // 32 * 8], 0.8 * (hi - lo) / steps, 0.03)
                    if k1 == edges[-1]:
                        for j, i in enumerate(tiles):
                            m_s[i] = m[:, j * T:(j + 1) * T]
                    yield
        blk.matmuls(gen(), 2 * steps, lo, hi)

    def spread_q(h):
        def gen(i):
            for d in range(0, DH, 8):
                q = qt_s[i, _rows(h & 15, DH), :].astype(F32)[d:d + 8]
                for n in range(8):
                    qb_s[i, _rows(d + n, 8), :] = jnp.broadcast_to(q[n:n + 1], (8, T))
                yield
        return [_Job(gen(i), DH // 8, 1, (qb_s, 0), None) for i in range(NT)]

    def vector_scores(keys):
        made = []

        def gen(tiles, group):
            s = {}
            for d in range(DH):
                k = jnp.concatenate([kb_s[group + n, _rows(d, 8), :] for n in (1, 0)], axis=0)
                for i in tiles:
                    q = qb_s[i, _rows(d, 8), :]
                    p = k * jnp.concatenate([q, q], axis=0)
                    s[i] = p if d == 0 else s[i] + p
                if d == DH - 1:
                    for i in tiles:
                        s_buf[i, S - 8 * group - 16:S - 8 * group, :] = s[i]
                        m_s[i] = _fold(s[i], jnp.maximum, m_s[i])
                if d % 4 == 3:
                    yield s[tiles[d // 4 % 2]][8 * (d // 8 % 2):]

        return [_Job(gen((i, i + 1), group), DH // 4, 1, (qb_s, 0), (s_buf, 0), 0.11, made)
                for i in range(0, NT, 2) for group in range(0, keys // 8, 2)]

    def weighted(blk, h, lo, hi, width):
        def gen():
            for first in range(0, NT, width):
                tiles = range(first, first + width)
                m = jnp.max(jnp.concatenate([m_s[i] for i in tiles], axis=1), axis=0, keepdims=True)
                o = total = None
                for kc in range(NT):
                    s = jnp.concatenate([s_buf[i, _rows(kc, T), :] for i in tiles], axis=1)
                    p = jnp.exp2(s - m)
                    total = _fold(p, jnp.add, total)
                    pv = _dot(_unpack(vt_s[kc]), p.astype(BF16))
                    o = pv if o is None else o + pv
                    if kc == NT - 1:
                        inv = 1.0 / jnp.sum(total, axis=0, keepdims=True)
                        for j, i in enumerate(tiles):
                            lanes = slice(j * T, (j + 1) * T)
                            ot_s[i, _rows(h & 15, DH), :] = (
                                o[:, lanes] * (inv[:, lanes] * gt_s[i][0:1]))
                    yield
        blk.matmuls(gen(), NT // width * NT, lo, hi)

    def head(blk, h, lo, hi, width, later):
        lead = 0.25 * (hi - lo) / (NT // width * NT)
        weighted(blk, h, lo + lead, hi + lead, width)
        scores(blk, h + 1, lo, hi, width, later)
        if later:
            blk.jobs(lo + 0.05, hi - 0.3, spread_q(h + 1))

    def q_transpose(items):
        def gen(tile, group):
            qt_s[tile, _rows(group & 3, T), :] = qo_s[tile, group, 0:T, :].T.astype(BF16)
            yield
        return [_Job(gen(n & 15, n >> 4), 1, 70, (qo_s, 0, 0), (qt_s, NT), TRANSPOSE_LAG)
                for n in items]

    def o_transpose(items):
        def gen(tile, group):
            qo_s[tile, group, 0:T, :] = ot_s[tile, _rows(group & 3, T), :].T
            yield
        return [_Job(gen(n & 15, n >> 4), 1, 70, (ot_s, NT), (qo_s, 0, 0), TRANSPOSE_LAG)
                for n in items]

    def x_operands(c):
        def block(a, n, j):
            return x_v[c][a, _rows(j, 16), n * T:(n + 1) * T].astype(F32)
        return row_operands(c, block, (x_v[c], 4), OPERAND_COST)

    def kv_projection(blk, *chunks):
        scale = DH ** -0.5 * math.log2(math.e)
        for c in chunks:
            for a in range(4):
                kvg = lax.dot_general(wkv[...], x_v[c][a], (((1,), (1,)), ((), ())),
                                      preferred_element_type=F32)
                blk.note(kvg[0:8], 0.05)
                g = jax.nn.sigmoid(kvg[2 * DH:2 * DH + 8])
                tile = 4 * c + a
                vt_s[tile] = _pack(kvg[DH:2 * DH])
                gt_s[tile] = g
                by_row = jnp.concatenate(
                    [kvg[0:DH] * scale, 1.0 - g, jnp.zeros((T - DH - 8, T), F32)], axis=0).T
                k_s[_rows(tile, T // 2), :] = _pack(by_row)
                gc_s[tile] = jnp.broadcast_to(by_row[:, DH:DH + 1], (T, T))
                for j in range(T // 8):
                    group = (S - tile * T) // 8 - 1 - j
                    if group < VECTOR_KEYS // 8:
                        for d in range(DH):
                            kb_s[group, _rows(d, 8), :] = jnp.broadcast_to(
                                by_row[8 * j:8 * j + 8, d:d + 1], (8, T))
                yield

    def q_results(side, c, out=None):
        def finish(a, b, rows, v):
            qo_s[4 * c + a, 4 * side + b, rows, :] = v
        return results((rl, rr)[side if out is None else out], finish, (qo_s, 0, 0))

    def arrive(done, more):
        _wait(done)
        _start(more)
        yield

    def just_ahead(blk, jobs, lo, early=0.0):
        def gen(some):
            for job in some:
                next(job.gen)
                yield

        def settle():
            blk.barrier(jobs[0].dst)
            yield

        blk.at(lo - early, _whole(gen(jobs)))
        for u in range(1, 7):
            blk.jobs(lo + (u - 1) / 7, lo + (u - 0.312) / 7,
                     [_Job(gen(jobs[k:k + 4]), 4, 1, jobs[0].src, None) for k in range(0, 16, 4)])
            blk.at(lo + u / 7 - 1e-4, settle())

    x_copies = [pltpu.make_async_copy(x_hbm.at[pl.ds(4 * c, 4)], x_v[c].at[pl.ds(0, 4)],
                                      x_sem.at[c]) for c in range(NCH)]
    wq_copies = side_copies(0, wq_hbm)
    small = [pltpu.make_async_copy(wkt_hbm, wkv.at[pl.ds(0, DH)], sem),
             pltpu.make_async_copy(wvt_hbm, wkv.at[pl.ds(DH, DH)], sem),
             pltpu.make_async_copy(gw_hbm, gw_v, sem)]
    _start(small + x_copies[:1] + wq_copies[:1])
    _wait(small)
    gw = gw_v[...].astype(F32)
    wkv[2 * DH:, :] = jnp.concatenate(
        [jnp.broadcast_to(gw[n:n + 1], (16, T)) for n in range(D // T)], axis=1).astype(BF16)
    zero = _zero(lax.bitcast_convert_type(gw, jnp.int32)[0, 0])

    x_copies[0].wait()
    x_copies[1].start()
    blk = _Block(zero)
    blk.matmuls(kv_projection(blk, 0), 4, 0, 0.2)
    blk.jobs(0, 0.3, [_Job(_whole(job.gen), 1, 1, job.dst, None) for job in x_operands(0)])
    blk.run()

    blk = _Block(zero, 0.103)
    blk.at(0, arrive(wq_copies[:1], wq_copies[1:] + x_copies[2:3]))
    just_ahead(blk, side_operands(0, 0, 0, 16), 0)
    products(blk, 0, 0, 0, 0)
    blk.at(1, arrive(x_copies[1:2], x_copies[3:]))
    just_ahead(blk, x_operands(1), 1)
    products(blk, 0, 0, 1, 1, out=1)
    blk.jobs(1 + 0.101, 1 + 0.93, q_results(0, 0))
    blk.at(2, arrive(wq_copies[1:] + x_copies[2:3], side_copies(1)))
    just_ahead(blk, side_operands(1, 0, 0, 16), 2.4, 0.3)
    blk.matmuls(kv_projection(blk, 1, 2), 8, 2, 2.39)
    products(blk, 1, 0, 0, 2.4, again=True, out=0)
    blk.jobs(2.054, 2.3, q_results(0, 1, out=1))
    products(blk, 1, 0, 1, 3.4, again=True)
    blk.jobs(3.428, 4.299, q_results(1, 0, out=0), x_operands(2))
    blk.at(4.4, arrive(x_copies[3:] + side_copies(1), side_copies(2) + down_copies(1)))
    blk.matmuls(kv_projection(blk, 3), 4, 4.8, 4.99)
    for c in (2, 3):
        products(blk, 0, 0, c, 2 * c + 1)
        products(blk, 1, 0, c, 2 * c + 2, again=True)
    jobs = x_operands(3)
    blk.jobs(5, 6 - 0.123, q_results(1, 1), jobs[:10])
    blk.jobs(6.06, 6.932, q_results(0, 2), jobs[10:])
    blk.jobs(7.06, 7.93, q_results(1, 2), side_operands(1, 1, 0, 6))
    blk.jobs(8.06, 8.98, q_results(0, 3), side_operands(0, 1, 0, 6))
    blk.jobs(8.0, 8.75, q_transpose(range(12)))
    scores(blk, 0, 9, 11.6, 4)
    blk.jobs(9.06, 11.4, q_results(1, 3), side_operands(0, 1, 6, 10),
             side_operands(1, 1, 6, 10))
    blk.jobs(9.0, 11.2, q_transpose(range(12, 40)))
    blk.run()

    def gates(c):
        tiles = [4 * c + a for a in range(4)]

        def finish(a, b, rows, v):
            g_buf[4 * a + b, rows, :] = jnp.maximum(v, 0.0) * gc_s[tiles[a], rows, :]
        return results(rl, finish, (g_buf, 0))

    def ups():
        def finish(a, b, rows, v):
            h_buf[4 * a + b, rows, :] = v * g_buf[4 * a + b, rows, :]
        return results(rr, finish, (h_buf, 0))

    def h_operands():
        def job(rows):
            def emit(t, v):
                ha[t, rows, :] = v.astype(BF16)

            return _Job(_operands(_LEFT, lambda a, b: h_buf[4 * a + b, rows, :], emit),
                        7, 206, (h_buf, 0), (ha, NP))
        return [job(slice(16 * j, 16 * j + 16)) for j in range(T // 16)]

    def down_products(blk, i, lo):
        slot, rows = ((i >> 2) + 1) & 1, _rows(i & 3, T)

        def gen():
            for t in range(NP):
                b = jnp.concatenate([_unpack(wd[slot, 2 * t + side, 0:T // 2, :])
                                     for side in (0, 1)], axis=1)
                res = _dot(ha[t, 0:T, :], b)
                for side in (0, 1):
                    acc[2 * t + side, rows, :] += res[:, side * T:(side + 1) * T]
                if t % 2 == 0:
                    blk.note(res, 2 / NP)
                yield
        blk.matmuls(gen(), NP, lo, lo + 1, (wd, 0, 2 * NP))

    def ffn_step(blk, i, alone=False):
        quad, c = (i >> 2) + 1, i & 3
        quad_d, c_d = ((i - 2) >> 2) + 2, (i - 2) & 3
        products(blk, 0, quad, c, 0)
        down_products(blk, i - 2, 1)
        products(blk, 1, quad, c, 2, again=True)
        work = dict(U=ups(), G=gates(c), H=h_operands(),
                    L=side_operands(0, quad + 1, 4 * c, 4), R=side_operands(1, quad + 1, 4 * c, 4),
                    D=[] if alone else down_operands(jnp.minimum(quad_d, NQ), quad_d, 2 * c_d, 4))
        for names, lo, hi in STEP_PLAN:
            lists = []
            for k in dict.fromkeys(names):
                n = len(work[k]) if k in "UGH" else names.count(k)
                lists.append(work[k][:n])
                work[k] = work[k][n:]
            blk.jobs(*((0.0, 0.9) if alone and lo < 0 else (lo, hi)), *lists)
        assert not any(work.values())

    last = NQ * NCH - 1
    offset = H - 1 - last

    _wait(side_copies(2) + down_copies(1))
    _start(down_copies(2))
    blk = _Block(zero, 0.112)
    head(blk, 0, -3.3, 0, 2, 64)
    blk.jobs(0, 2.03, vector_scores(64))
    products(blk, 0, 1, 0, 0)
    products(blk, 1, 1, 0, 1, again=True)
    jobs = down_operands(1, 1, 0, 16)
    blk.jobs(-3.1, -0.2, jobs[:8])
    blk.jobs(0, 0.95, jobs[8:])
    blk.jobs(1.06, 1.93, gates(0), side_operands(0, 2, 0, 8))
    blk.run()

    _wait(down_copies(2))
    blk = _Block(zero, 0.112)
    head(blk, 1, -3.3, 0, 2, 64)
    blk.jobs(0, 2.03, vector_scores(64))
    products(blk, 0, 1, 1, 0)
    products(blk, 1, 1, 1, 1, again=True)
    blk.jobs(-3.1, -0.2, side_operands(1, 2, 4, 4))
    blk.jobs(0, 0.9, ups(), side_operands(1, 2, 0, 4))
    blk.jobs(1.06, 1.96, gates(1), h_operands())
    blk.jobs(0.1, 1.6, q_transpose(range(40, 48)))
    blk.run()

    def head_only(h, carry):
        def clear(tile):
            for row in range(0, NCH * T, T // 2):
                acc[tile, row:row + T // 2, :] = jnp.zeros((T // 2, T), F32)
                yield

        blk = _Block(_zero(h))
        head(blk, h, 0, 3.3, 2, 0)
        count = -(-2 * NP // offset)
        blk.jobs(0.03, 3.25, [_Job(clear(jnp.minimum((h - 2) * count + k, 2 * NP - 1)), 2 * NCH, 1,
                                   (acc, 2 * NP), None) for k in range(count)])
        blk.run()
        return carry

    lax.fori_loop(2, 2 + offset, head_only, 0)

    def step(i, carry):
        blk = _Block(_zero(i))
        head(blk, i + offset, -3.3, 0, 4, VECTOR_KEYS)
        jobs = vector_scores(VECTOR_KEYS)
        shares = (1.0, 0.991, 1.025)
        for k, share in enumerate(shares):
            n = round(len(jobs) * share / sum(shares[k:]))
            blk.jobs(k, k + 1, jobs[:n])
            jobs = jobs[n:]
        items = [4 * (i - 2) + k for k in range(4)]
        blk.jobs(0.06, 2.568, o_transpose(items)
                 + q_transpose([jnp.minimum(48 + n, 8 * NT - 1) for n in items]))
        ffn_step(blk, i)
        blk.run()
        return carry

    def quad_steps(quad, carry):
        pl.when((quad > 1) & (quad < NQ))(
            lambda: _wait(side_copies(quad + 1) + down_copies(quad + 1)))
        pl.when(quad < NQ - 1)(lambda: _start(side_copies(quad + 2) + down_copies(quad + 2)))
        pl.when(quad == NQ - 1)(lambda: _start(side_copies(NQ + 1, wo_hbm)))
        pl.when(quad == NQ)(lambda: _wait(side_copies(NQ + 1, wo_hbm)))
        return lax.fori_loop(jnp.maximum(4 * quad - 4, 2), jnp.minimum(4 * quad, last), step, carry)

    lax.fori_loop(1, NQ + 1, quad_steps, 0)

    blk = _Block(zero, 0.106)
    ffn_step(blk, last, alone=True)
    weighted(blk, H - 1, -0.02, 2.504, 2)
    blk.jobs(0.1, 0.9, o_transpose(range(100, 112)))
    blk.jobs(1.0, 1.2, o_transpose(range(112, 116)))
    blk.jobs(1.7, 1.9, o_transpose(range(116, 120)))
    blk.jobs(2.3, 2.5, o_transpose(range(120, 124)))
    blk.run()

    def o_operands(c):
        def block(a, n, j):
            return qo_s[4 * c + a, n, _rows(j, 16), :]
        return row_operands(c, block, (qo_s, 0, 0), 200)

    def o_products(side, c, lo):
        products(blk, side, NQ + 1, c, lo, again=side == 1,
                 base=lambda t: acc[2 * t + side, _rows(c, T), :])

    def outputs(side, c):
        def finish(a, b, rows, v):
            row = side * CH + a * T
            raw[c, row + rows.start:row + rows.stop, b * T:(b + 1) * T] = v.astype(BF16)
        return results((rl, rr)[side], finish, raw_spare)

    sent = []

    def send(c, side, parts=((0, CH),)):
        copies = [pltpu.make_async_copy(raw.at[c, pl.ds(side * CH + row, n)],
                                        out_hbm.at[pl.ds(c * CH + row, n), pl.ds(side * CH, CH)],
                                        sem) for row, n in parts]
        _start(copies)
        sent.extend(copies)
        yield

    blk = _Block(zero, 0.103)
    down_products(blk, last - 1, 0)
    o_products(0, 0, 1)
    o_products(1, 0, 2)
    down_products(blk, last, 3)
    jobs = o_operands(1)
    blk.jobs(0.043, 0.943, o_operands(0))
    blk.jobs(1.0, 1 + 0.897, ups(), jobs[:10])
    blk.jobs(2.06, 2.92, outputs(0, 0), h_operands())
    blk.jobs(2.1, 2.6, o_transpose(range(124, 128)))
    blk.jobs(3.06, 3 + 0.906, outputs(1, 0), jobs[10:])
    for c in range(1, NCH):
        lo = 2 * c + 2
        o_products(0, c, lo)
        o_products(1, c, lo + 1)
        jobs = o_operands(c + 1) if c + 1 < NCH else []
        cut = 9 if c > 1 else 8
        blk.jobs(lo + 0.06, lo + (0.897 if jobs else 0.906), outputs(1, c - 1) if c > 1 else [],
                 jobs[:cut])
        blk.jobs(lo + 1.06, lo + 1 + (0.906 if jobs else 0.785), outputs(0, c), jobs[cut:])
        blk.at(lo + 0.05, send(c - 1, 0))
        blk.at(lo + 1.05, send(c - 1, 1))
    blk.at(lo + 1.85, send(NCH - 1, 0))
    blk.run()
    for j, job in enumerate(outputs(1, NCH - 1)):
        next(_whole(job.gen))
        if j % 8 == 7:
            next(send(NCH - 1, 1, [(a * T + 8 * j - 56, T // 2) for a in range(4)]))
    _wait(sent)


@jax.jit
def pallas_gated_mix__grouped_kv_mqa__glu_gated_reglu__prompt_kernel(
        A_x, A_wq, A_wk, A_wv, A_wo, B_x, B_W_gate, B_W_up, B_W_down, gate_w):
    del B_x
    hbm = pl.BlockSpec(memory_space=pl.ANY)
    operands = pltpu.VMEM((2, 2 * NP + 2, T // 2 + 8, T), U32)
    block_products = pltpu.VMEM((NP + 3, T + 8, T), F32)
    blocks = pltpu.VMEM((16, T + 8, T), F32)
    out = pl.pallas_call(
        _kernel,
        out_shape=jax.ShapeDtypeStruct((S, D), BF16),
        in_specs=[hbm] * 9,
        out_specs=hbm,
        scratch_shapes=[
            pltpu.VMEM((9, D, CH), BF16),
            pltpu.VMEM((2 * NP + 2, NCH * T // 2 + 8, T), U32),
            operands, operands, operands,
            block_products, block_products, blocks, blocks,
            pltpu.VMEM((NP + 3, T + 16, T), BF16),
            pltpu.VMEM((2 * NP + 2, NCH * T + 8, T), F32),
            pltpu.VMEM((S // 2, T), U32),
            pltpu.VMEM((NT, DH // 2, T), U32),
            pltpu.VMEM((NT, 8, T), F32),
            pltpu.VMEM((NT, T, T), F32),
            pltpu.VMEM((NT + 1, 4 * T, T), BF16),
            pltpu.VMEM((NT, 8, T), F32),
            pltpu.VMEM((NT + 1, 4 * T, T), F32),
            pltpu.VMEM((NT, 8, T + 8, T), F32),
            pltpu.VMEM((NT, S + 8, T), F32),
            pltpu.VMEM((-(-VECTOR_KEYS // 32) * 4, 8 * DH + 8, T), F32),
            pltpu.VMEM((NT, 8 * DH + 8, T), F32),
            [pltpu.VMEM((5, T, D), BF16)] * NCH,
            pltpu.VMEM((2 * DH + 16, D), BF16),
            pltpu.VMEM((D // T, T), BF16),
            pltpu.SemaphoreType.DMA((NCH,)),
            pltpu.SemaphoreType.DMA((6,)),
            pltpu.SemaphoreType.DMA(()),
        ],
        compiler_params=pltpu.CompilerParams(vmem_limit_bytes=127 * 2 ** 20,
                                             internal_scratch_in_bytes=96 * 512),
        name="gated_mix",
    )(A_x.reshape(NT, T, D), A_wq, A_wk.T, A_wv.T, A_wo, B_W_gate, B_W_up, B_W_down,
      gate_w.reshape(D // T, T))
    return out.reshape(1, S, D)
```
